```python
import os as _os
_os.environ.setdefault("JAX_PLATFORMS", "cpu")
import jax
import jax.numpy as jnp

def _softmax(x, axis=-1):
    return jax.nn.softmax(x, axis=axis)
def _gelu(x):
    return jax.nn.gelu(x, approximate=True)
def _silu(x):
    return jax.nn.silu(x)
def _sigmoid(x):
    return jax.nn.sigmoid(x)
def _layernorm(x, axis=-1, eps=1e-5):
    m = jnp.mean(x, axis=axis, keepdims=True)
    v = jnp.var(x, axis=axis, keepdims=True)
    return (x - m) / jnp.sqrt(v + eps)
def _scatter_add(tgt, idx, src, axis=0):
    return tgt.at[idx].add(src)
def _segment_sum(src, seg, n):
    return jax.ops.segment_sum(src, seg, n)
class _Rng:
    def __init__(self, key):
        self._k = key
    def _next(self):
        self._k, sub = jax.random.split(self._k)
        return sub
    def normal(self, shape):
        return jax.random.normal(self._next(), shape, dtype=jnp.bfloat16)
    def randint(self, lo, hi, shape):
        return jax.random.randint(self._next(), shape, lo, hi, dtype=jnp.int32)
    def uniform(self, shape, lo=0.0, hi=1.0):
        return jax.random.uniform(self._next(), shape, jnp.bfloat16, lo, hi)
    def permutation(self, n):
        return jax.random.permutation(self._next(), n)


kernel_name = 'standalone__gqa_block_cached__near_ridge'

def setup_inputs():
    _rng = _Rng(jax.random.key(int.from_bytes(__import__("os").urandom(4), "little")))
    _w = (lambda a: (lambda t: t.astype(jnp.bfloat16) if jnp.issubdtype(t.dtype, jnp.floating) else t)(jnp.asarray(a)))
    B, Sq, D = 16, 128, 576
    Hq, Hkv, Sk, Dh = 32, 16, 1024, 128
    assert Hq % Hkv == 0, (Hq, Hkv)
    return {
        "x": _w((lambda *s: _rng.normal(s) * 0.8)(B, Sq, D)),
        "k_cache": _w((lambda *s: _rng.normal(s) * 0.8)(B, Hkv, Sk, Dh)),
        "v_cache": _w((lambda *s: _rng.normal(s) * 0.05)(B, Hkv, Sk, Dh)),
        "wq": _w((lambda *s: _rng.normal(s) * 0.8)(D, Hq * Dh) * (D ** -0.5)),
        "wo": _w((lambda *s: _rng.normal(s) * 0.05)(Hq * Dh, D) * ((Hq * Dh) ** -0.5)),
    }

def reference(x, k_cache, v_cache, wq, wo):
    B, Sq, D = x.shape
    Hq, Dh = 32, 128
    Hkv = k_cache.shape[1]
    rep = Hq // Hkv
    q = (lambda x, *d: x.transpose(*d))((x @ wq).reshape(B, Sq, Hq, Dh), 0, 2, 1, 3)
    k = jnp.repeat(k_cache, rep, axis=1)
    v = jnp.repeat(v_cache, rep, axis=1)
    scores = jnp.einsum("bhqd,bhkd->bhqk", q, k) * (Dh ** -0.5)
    p = _softmax(scores, axis=-1)
    o = jnp.einsum("bhqk,bhkd->bhqd", p, v)
    return (lambda x, *d: x.transpose(*d))(o, 0, 2, 1, 3).reshape(B, Sq, Hq * Dh) @ wo
```

```python
import jax
import jax.numpy as jnp
import numpy as np
import jax.experimental.pallas as pl
import jax.experimental.pallas.tpu as pltpu

G = 4
U = 4
ORDER = "qk0 xt0 sm0 qk1 qp0 pv0 qp1 qk2 op0 sm1 pv1 op1 qk3 sm3 sm2 pv2 pv3".split()


@jax.jit
def pallas_standalone__gqa_block_cached__near_ridge_kernel(x, k_cache, v_cache, wq, wo):
    B, Sq, D = x.shape
    _, Hkv, Sk, Dh = k_cache.shape
    Hq = wq.shape[1] // Dh
    rep = Hq // Hkv
    NC = Hkv // G
    W = G * rep * Dh
    NS = B * NC
    LB = B.bit_length() - 1
    assert G == 4 and wq.dtype == wo.dtype and B == 1 << LB and Hkv % G == 0 and U % 2 == 0 and B % U == 0 and B > 3 * U + 2 and NC >= 2
    qscale = float(Dh ** -0.5 * np.log2(np.e))
    NT = (((1,), (1,)), ((), ()))
    f32, bf16 = jnp.float32, jnp.bfloat16
    XH, XA, XM = 3, U + 2, 3 * U + 2

    def kernel(xt_hbm, k_hbm, v_hbm, wq_hbm, wot_hbm, out_hbm,
               xt_buf, k_buf, v_buf, w_buf, out_buf,
               q_scr, o_scr, acc_ref, x_scr, sem_k, sem_v, sem_w, sem_x, sem_out):

        def k_copy(s, slot, j):
            return pltpu.make_async_copy(k_hbm.at[s & (B - 1), (s >> LB) * G + j], k_buf.at[slot, j], sem_k.at[slot, j])

        def v_copy(s, slot, j):
            return pltpu.make_async_copy(v_hbm.at[s & (B - 1), (s >> LB) * G + j], v_buf.at[slot, j], sem_v.at[slot, j])

        def kv_start(s, slot):
            for kind, j in KV_ISSUE:
                (k_copy if kind == 'k' else v_copy)(s, slot, j).start()

        def cols(c, lo, n):
            return pl.ds(pl.multiple_of(c * W + lo, 128), n)

        def wq_copy(c):
            return pltpu.make_async_copy(wq_hbm.at[:, cols(c, 0, W)], w_buf.at[c], sem_w.at[0])

        def wq0_copy(h):
            sl = pl.ds(pl.multiple_of(h * (W // 2), 128), W // 2)
            return pltpu.make_async_copy(wq_hbm.at[:, sl], w_buf.at[0, :, sl], sem_w.at[2 + h])

        def wot0_copy(h):
            sl = pl.ds(pl.multiple_of(h * (W // 2), 128), W // 2)
            return pltpu.make_async_copy(wot_hbm.at[:, sl], w_buf.at[NC, :, sl], sem_w.at[4 + h])

        def wot_copy(c):
            return pltpu.make_async_copy(wot_hbm.at[:, cols(c, 0, W)], w_buf.at[NC + c], sem_w.at[1])

        def x_copy(i):
            return pltpu.make_async_copy(xt_hbm.at[pl.ds(i, 1)], xt_buf.at[pl.ds(i, 1)], sem_x.at[i])

        def x_range(lo, hi, i):
            return pltpu.make_async_copy(xt_hbm.at[pl.ds(lo, hi - lo)], xt_buf.at[pl.ds(lo, hi - lo)], sem_x.at[XH + i])

        x_a, x_mid, x_rest = x_range(XH, XA, 0), x_range(XA, XM, 1), x_range(XM, B, 2)

        def out_copy(b):
            return pltpu.make_async_copy(out_buf.at[b], out_hbm.at[b], sem_out)

        def q_proj(slot_x, c, slot_q, lo, n):
            q = jnp.dot(x_scr[slot_x], w_buf[c, :, lo:lo + n], preferred_element_type=f32)
            q_scr[slot_q, :, lo:lo + n] = (q * qscale).astype(bf16)

        def o_proj(wi, slot_o, lo, n):
            return jax.lax.dot_general(w_buf[wi, :, lo:lo + n], o_scr[slot_o, :, lo:lo + n], NT,
                                       preferred_element_type=f32)

        def run_step(s, cur):
            nxt = 1 - cur
            sp = jnp.maximum(s - 1, 0)
            bp, cp = sp & (B - 1), sp >> LB
            wi = jnp.where(s == 0, 0, NC + cp)
            cn = jnp.minimum((s + 1) >> LB, NC - 1)
            nop = sum(t.startswith('op') for t in ORDER)
            nqp = sum(t.startswith('qp') for t in ORDER)
            st = {}
            for t in ORDER:
                kind, j = t[:2], int(t[2:])
                if kind == 'qk':
                    k_copy(s, cur, j).wait()
                    q = jnp.concatenate([q_scr[cur, :, (j * rep + r) * Dh:(j * rep + r + 1) * Dh] for r in range(rep)], axis=0)
                    st['s', j] = jax.lax.dot_general(q, k_buf[cur, j], NT, preferred_element_type=f32)
                elif kind == 'sm':
                    sc = st.pop(('s', j))
                    m = jnp.max(sc, axis=-1, keepdims=True)
                    p = jnp.exp2(sc - m)
                    st['l', j] = jnp.sum(p, axis=-1, keepdims=True)
                    st['p', j] = p.astype(bf16)
                elif kind == 'pv':
                    v_copy(s, cur, j).wait()
                    o = jnp.dot(st.pop(('p', j)), v_buf[cur, j], preferred_element_type=f32)
                    l = st.pop(('l', j))
                    r = pl.reciprocal(l, approx=True)
                    r = r * (2.0 - l * r)
                    o = (o * r).astype(bf16)
                    for h in range(rep):
                        o_scr[cur, :, (j * rep + h) * Dh:(j * rep + h + 1) * Dh] = o[h * Sq:(h + 1) * Sq]
                elif kind == 'op':
                    n = W // nop
                    if j == 0:
                        if cur == 1:
                            @pl.when(s == 1)
                            def _():
                                for h in range(2):
                                    wot0_copy(h).wait()
                        st['acc'] = jnp.where(cp == 0, 0.0, acc_ref[bp])
                    st['acc'] = st['acc'] + o_proj(wi, nxt, j * n, n)
                    if j == nop - 1:
                        acc = st.pop('acc')
                        acc_ref[bp] = acc
                        out_buf[bp] = acc.astype(out_buf.dtype)
                elif kind == 'qp':
                    n = W // nqp
                    q_proj(cur, cn, nxt, j * n, n)
                elif kind == 'xt':
                    if cur == 1:
                        pl.when(s == 1)(lambda: x_a.wait())
                    x_scr[nxt] = xt_buf[(s + 2) & (B - 1)].T
            pl.when(s + 2 < NS)(lambda: kv_start(s + 2, cur))

        def loop(n, fn):
            jax.lax.fori_loop(0, n, lambda i, c: (fn(i), c)[1], 0)

        x_copy(0).start()
        loop(2, lambda h: wq0_copy(h).start())
        loop(XH - 1, lambda i: x_copy(1 + i).start())
        loop(1, lambda j: k_copy(0, 0, j).start())
        loop(1, lambda j: v_copy(0, 0, j).start())
        loop(2, lambda j: k_copy(0, 0, 1 + j).start())
        loop(1, lambda j: v_copy(0, 0, 1 + j).start())
        loop(1, lambda j: k_copy(0, 0, 3 + j).start())
        loop(2, lambda j: v_copy(0, 0, 2 + j).start())
        loop(2, lambda j: k_copy(1, 1, j).start())
        x_a.start()
        loop(1, lambda j: k_copy(1, 1, 2 + j).start())
        loop(2, lambda j: v_copy(1, 1, j).start())
        loop(2, lambda h: wot0_copy(h).start())
        loop(1, lambda j: k_copy(1, 1, 3 + j).start())
        loop(2, lambda j: v_copy(1, 1, 2 + j).start())
        o_scr[1] = jnp.zeros(o_scr.shape[1:], o_scr.dtype)

        def zero_acc(b):
            acc_ref[b] = jnp.zeros(acc_ref.shape[1:], acc_ref.dtype)
        loop(B, zero_acc)

        loop(1, lambda i: x_copy(i).wait())
        x_scr[1] = xt_buf[0].T

        def first_q(h):
            wq0_copy(h).wait()
            sl = pl.ds(pl.multiple_of(h * (W // 2), 128), W // 2)
            q = jnp.dot(x_scr[1], w_buf[0, :, sl], preferred_element_type=f32)
            q_scr[0, :, sl] = (q * qscale).astype(bf16)
        loop(2, first_q)
        loop(XH - 1, lambda i: x_copy(1 + i).wait())
        x_scr[0] = xt_buf[1].T
        x_mid.start()

        def weights_prefetch(s0):
            b0, c0 = s0 & (B - 1), s0 >> LB
            more = c0 + 1 < NC

            @pl.when(jnp.logical_and(b0 == U, more))
            def _():
                wq_copy(c0 + 1).start()
                wot_copy(c0 + 1).start()

            @pl.when(jnp.logical_and(b0 == B - 2 * U, more))
            def _():
                wq_copy(c0 + 1).wait()
                wot_copy(c0 + 1).wait()

        F = (NC - 1) * B

        def iteration(i, carry):
            s0 = i * U
            weights_prefetch(s0)
            pl.when(s0 == U)(lambda: x_mid.wait())
            pl.when(s0 == 2 * U)(lambda: x_rest.start())
            pl.when(s0 == 3 * U)(lambda: x_rest.wait())
            for u in range(U):
                run_step(s0 + u, u % 2)

            @pl.when(s0 > F)
            def _():
                for u in range(U):
                    out_copy(s0 - 1 - F + u).start()

            @pl.when(s0 == F)
            def _():
                for u in range(1, U):
                    out_copy(u - 1).start()
            return carry

        jax.lax.fori_loop(0, NS // U, iteration, 0)

        r = o_proj(2 * NC - 1, (NS - 1) % 2, 0, W)
        out_buf[B - 1] = (acc_ref[B - 1] + r).astype(out_buf.dtype)
        out_copy(B - 1).start()
        for b in range(B):
            out_copy(b).wait()

    KV_ISSUE = [('k', 0), ('k', 1), ('v', 0), ('k', 2), ('v', 1), ('k', 3), ('v', 2), ('v', 3)]
    xT = jnp.transpose(x, (0, 2, 1))
    woT = wo.T
    hbm = pl.BlockSpec(memory_space=pl.ANY)
    outT = pl.pallas_call(
        kernel,
        in_specs=[hbm] * 5,
        out_specs=hbm,
        out_shape=jax.ShapeDtypeStruct((B, D, Sq), x.dtype),
        scratch_shapes=[
            pltpu.VMEM((B, D, Sq), x.dtype), pltpu.VMEM((2, G, Sk, Dh), k_cache.dtype), pltpu.VMEM((2, G, Sk, Dh), v_cache.dtype),
            pltpu.VMEM((2 * NC, D, W), wq.dtype), pltpu.VMEM((B, D, Sq), x.dtype),
            pltpu.VMEM((2, Sq, W), bf16), pltpu.VMEM((2, Sq, W), bf16), pltpu.VMEM((B, D, Sq), f32), pltpu.VMEM((2, Sq, D), bf16),
            pltpu.SemaphoreType.DMA((2, G)), pltpu.SemaphoreType.DMA((2, G)), pltpu.SemaphoreType.DMA((6,)),
            pltpu.SemaphoreType.DMA((XH + 3,)), pltpu.SemaphoreType.DMA(()),
        ],
        compiler_params=pltpu.CompilerParams(
            vmem_limit_bytes=100 * 1024 * 1024, disable_bounds_checks=True,
            flags={"XLA_TPU_RESCHEDULE_DMA_DONES": True}),
    )(xT, k_cache, v_cache, wq, woT)
    return jnp.transpose(outT, (0, 2, 1))
```
